```python
import os as _os
_os.environ.setdefault("JAX_PLATFORMS", "cpu")
import jax
import jax.numpy as jnp

def _softmax(x, axis=-1):
    return jax.nn.softmax(x, axis=axis)
def _gelu(x):
    return jax.nn.gelu(x, approximate=True)
def _silu(x):
    return jax.nn.silu(x)
def _sigmoid(x):
    return jax.nn.sigmoid(x)
def _layernorm(x, axis=-1, eps=1e-5):
    m = jnp.mean(x, axis=axis, keepdims=True)
    v = jnp.var(x, axis=axis, keepdims=True)
    return (x - m) / jnp.sqrt(v + eps)
def _scatter_add(tgt, idx, src, axis=0):
    return tgt.at[idx].add(src)
def _segment_sum(src, seg, n):
    return jax.ops.segment_sum(src, seg, n)
class _Rng:
    def __init__(self, key):
        self._k = key
    def _next(self):
        self._k, sub = jax.random.split(self._k)
        return sub
    def normal(self, shape):
        return jax.random.normal(self._next(), shape, dtype=jnp.bfloat16)
    def randint(self, lo, hi, shape):
        return jax.random.randint(self._next(), shape, lo, hi, dtype=jnp.int32)
    def uniform(self, shape, lo=0.0, hi=1.0):
        return jax.random.uniform(self._next(), shape, jnp.bfloat16, lo, hi)
    def permutation(self, n):
        return jax.random.permutation(self._next(), n)


kernel_name = 'concat_heads__sliding_block_cached__sliding_block_cached__decode'

def setup_inputs():
    _rng = _Rng(jax.random.key(int.from_bytes(__import__("os").urandom(4), "little")))
    _w = (lambda a: (lambda t: t.astype(jnp.bfloat16) if jnp.issubdtype(t.dtype, jnp.floating) else t)(jnp.asarray(a)))
    def _A_setup():
        B, Sq, D = 2, 1, 640
        Hq, Hkv, Sk, Dh = 32, 32, 4096, 128
        assert Hq % Hkv == 0, (Hq, Hkv)
        return {
            "x": _w((lambda *s: _rng.normal(s) * 0.8)(B, Sq, D)),
            "k_cache": _w((lambda *s: _rng.normal(s) * 0.8)(B, Hkv, Sk, Dh)),
            "v_cache": _w((lambda *s: _rng.normal(s) * 0.05)(B, Hkv, Sk, Dh)),
            "wq": _w((lambda *s: _rng.normal(s) * 0.8)(D, Hq * Dh) * (D ** -0.5)),
            "wo": _w((lambda *s: _rng.normal(s) * 0.05)(Hq * Dh, D) * ((Hq * Dh) ** -0.5)),
        }
    _A_in = _A_setup()

    def _B_setup():
        B, Sq, D = 2, 1, 640
        Hq, Hkv, Sk, Dh = 32, 32, 4096, 128
        assert Hq % Hkv == 0, (Hq, Hkv)
        return {
            "x": _w((lambda *s: _rng.normal(s) * 0.8)(B, Sq, D)),
            "k_cache": _w((lambda *s: _rng.normal(s) * 0.8)(B, Hkv, Sk, Dh)),
            "v_cache": _w((lambda *s: _rng.normal(s) * 0.05)(B, Hkv, Sk, Dh)),
            "wq": _w((lambda *s: _rng.normal(s) * 0.8)(D, Hq * Dh) * (D ** -0.5)),
            "wo": _w((lambda *s: _rng.normal(s) * 0.05)(Hq * Dh, D) * ((Hq * Dh) ** -0.5)),
        }
    _B_in = _B_setup()

    return {
        "A_x": _A_in["x"],
        "A_k_cache": _A_in["k_cache"],
        "A_v_cache": _A_in["v_cache"],
        "A_wq": _A_in["wq"],
        "A_wo": _A_in["wo"],
        "B_x": _B_in["x"],
        "B_k_cache": _B_in["k_cache"],
        "B_v_cache": _B_in["v_cache"],
        "B_wq": _B_in["wq"],
        "B_wo": _B_in["wo"],
    }

def reference(A_x, A_k_cache, A_v_cache, A_wq, A_wo, B_x, B_k_cache, B_v_cache, B_wq, B_wo):
    def _A_ref(x, k_cache, v_cache, wq, wo):
        B, Sq, D = x.shape
        Hq, Dh = 32, 128
        Hkv, Sk = k_cache.shape[1], k_cache.shape[2]
        W = min(4096, max(256, Sk // 4))
        rep = Hq // Hkv
        q = (lambda x, *d: x.transpose(*d))((x @ wq).reshape(B, Sq, Hq, Dh), 0, 2, 1, 3)
        k = jnp.repeat(k_cache[:, :, Sk - W:, :], rep, axis=1)
        v = jnp.repeat(v_cache[:, :, Sk - W:, :], rep, axis=1)
        scores = jnp.einsum("bhqd,bhkd->bhqk", q, k) * (Dh ** -0.5)
        p = _softmax(scores, axis=-1)
        o = jnp.einsum("bhqk,bhkd->bhqd", p, v)
        return (lambda x, *d: x.transpose(*d))(o, 0, 2, 1, 3).reshape(B, Sq, Hq * Dh) @ wo

    def _B_ref(x, k_cache, v_cache, wq, wo):
        B, Sq, D = x.shape
        Hq, Dh = 32, 128
        Hkv, Sk = k_cache.shape[1], k_cache.shape[2]
        W = min(4096, max(256, Sk // 4))
        rep = Hq // Hkv
        q = (lambda x, *d: x.transpose(*d))((x @ wq).reshape(B, Sq, Hq, Dh), 0, 2, 1, 3)
        k = jnp.repeat(k_cache[:, :, Sk - W:, :], rep, axis=1)
        v = jnp.repeat(v_cache[:, :, Sk - W:, :], rep, axis=1)
        scores = jnp.einsum("bhqd,bhkd->bhqk", q, k) * (Dh ** -0.5)
        p = _softmax(scores, axis=-1)
        o = jnp.einsum("bhqk,bhkd->bhqd", p, v)
        return (lambda x, *d: x.transpose(*d))(o, 0, 2, 1, 3).reshape(B, Sq, Hq * Dh) @ wo

    a = _A_ref(A_x, A_k_cache, A_v_cache, A_wq, A_wo)
    b = _B_ref(B_x, B_k_cache, B_v_cache, B_wq, B_wo)
    return jnp.concatenate([a, b], axis=-1)
```

```python
import functools
import jax
import jax.numpy as jnp
from jax.experimental import pallas as pl
from jax.experimental.pallas import tpu as pltpu

H, DH, SK, W, D = 32, 128, 4096, 1024, 640
NSTEP = 2 * H


def make(name="attn_v1", depth=4):
    def kernel(xa, ka, va, wqa, woa, xb, kb, vb, wqb, wob, out,
               xbuf, wqbuf, qbuf, kbuf, vbuf, wobuf, acc, xsem, wqsem, ksem, vsem, wosem):
        xs, ks, vs, wqs, wos = (xa, xb), (ka, kb), (va, vb), (wqa, wqb), (woa, wob)

        x_c = [pltpu.make_async_copy(xs[i], xbuf.at[i], xsem.at[i]) for i in range(2)]
        wq_c = [pltpu.make_async_copy(wqs[i], wqbuf.at[i], wqsem.at[i]) for i in range(2)]

        def step_copies(br, h, slot):
            return (
                (pltpu.make_async_copy(ks[br].at[:, h, pl.ds(SK - W, W), :], kbuf.at[slot], ksem.at[slot]), 0),
                (pltpu.make_async_copy(vs[br].at[:, h, pl.ds(SK - W, W), :], vbuf.at[slot], vsem.at[slot]), 1),
                (pltpu.make_async_copy(wos[br].at[pl.ds(pl.multiple_of(h * DH, DH), DH), :], wobuf.at[slot], wosem.at[slot]), 0),
            )

        def start_step(i, slot):
            if isinstance(i, int):
                for c, p in step_copies(i // H, i % H, slot):
                    c.start(priority=p)
                return
            @pl.when(i < H)
            def _():
                for c, p in step_copies(0, i, slot):
                    c.start(priority=p)
            @pl.when(i >= H)
            def _():
                for c, p in step_copies(1, i - H, slot):
                    c.start(priority=p)

        wq_c[0].start()
        x_c[0].start()
        x_c[1].start()
        for i in range(depth):
            start_step(i, i)
        wq_c[1].start()

        scale = DH ** -0.5
        for br in range(2):
            x_c[br].wait()
            wq_c[br].wait()
            xv = xbuf[br]
            x16 = jnp.concatenate([jnp.broadcast_to(xv[0:1], (8, D)), jnp.broadcast_to(xv[1:2], (8, D))], axis=0)
            for h in range(H):
                q = jnp.dot(x16, wqbuf[br, :, h * DH:(h + 1) * DH], preferred_element_type=jnp.float32)
                qbuf[h] = q.astype(jnp.bfloat16)
            acc[...] = jnp.zeros_like(acc)

            def body(h, _, br=br):
                i = br * H + h
                slot = i % depth
                cs = step_copies(br, h, slot)
                q = qbuf[h]
                cs[0][0].wait()
                s0 = jax.lax.dot_general(q, kbuf[slot, 0], (((1,), (1,)), ((), ())), preferred_element_type=jnp.float32)
                s1 = jax.lax.dot_general(q, kbuf[slot, 1], (((1,), (1,)), ((), ())), preferred_element_type=jnp.float32)
                s = jnp.concatenate([s0[0:8], s1[8:16]], axis=0) * scale
                m = jnp.max(s, axis=-1, keepdims=True)
                p = jnp.exp(s - m)
                l = jnp.sum(p, axis=-1, keepdims=True)
                pb = p.astype(jnp.bfloat16)
                cs[1][0].wait()
                o0 = jnp.dot(pb, vbuf[slot, 0], preferred_element_type=jnp.float32)
                o1 = jnp.dot(pb, vbuf[slot, 1], preferred_element_type=jnp.float32)
                o = jnp.concatenate([o0[0:8], o1[8:16]], axis=0) / l
                cs[2][0].wait()
                acc[...] += jnp.dot(o.astype(jnp.bfloat16), wobuf[slot], preferred_element_type=jnp.float32)
                @pl.when(i + depth < NSTEP)
                def _():
                    start_step(i + depth, slot)
                return 0

            jax.lax.fori_loop(0, H, body, 0)
            a = acc[...]
            out[0:1, br * D:(br + 1) * D] = a[0:1].astype(out.dtype)
            out[1:2, br * D:(br + 1) * D] = a[8:9].astype(out.dtype)

    def f(xa, ka, va, wqa, woa, xb, kb, vb, wqb, wob):
        o = pl.pallas_call(
            kernel, name=name,
            out_shape=jax.ShapeDtypeStruct((2, 2 * D), jnp.bfloat16),
            in_specs=[pl.BlockSpec(memory_space=pl.ANY)] * 10,
            out_specs=pl.BlockSpec(memory_space=pltpu.VMEM),
            scratch_shapes=[
                pltpu.VMEM((2, 2, D), jnp.bfloat16),
                pltpu.VMEM((2, D, H * DH), jnp.bfloat16),
                pltpu.VMEM((H, 16, DH), jnp.bfloat16),
                pltpu.VMEM((depth, 2, W, DH), jnp.bfloat16),
                pltpu.VMEM((depth, 2, W, DH), jnp.bfloat16),
                pltpu.VMEM((depth, DH, D), jnp.bfloat16),
                pltpu.VMEM((16, D), jnp.float32),
                pltpu.SemaphoreType.DMA((2,)),
                pltpu.SemaphoreType.DMA((2,)),
                pltpu.SemaphoreType.DMA((depth,)),
                pltpu.SemaphoreType.DMA((depth,)),
                pltpu.SemaphoreType.DMA((depth,)),
            ],
            compiler_params=pltpu.CompilerParams(vmem_limit_bytes=100 * 1024 * 1024),
        )(xa.reshape(2, D), ka, va, wqa, woa, xb.reshape(2, D), kb, vb, wqb, wob)
        return o.reshape(2, 1, 2 * D)
    f.__name__ = name
    return f


_kernel_fn = make("concat_heads_sliding_decode", depth=3)


@jax.jit
def pallas_concat_heads__sliding_block_cached__sliding_block_cached__decode_kernel(
    A_x, A_k_cache, A_v_cache, A_wq, A_wo, B_x, B_k_cache, B_v_cache, B_wq, B_wo
):
    return _kernel_fn(A_x, A_k_cache, A_v_cache, A_wq, A_wo, B_x, B_k_cache, B_v_cache, B_wq, B_wo)
```

```python
import jax
import jax.numpy as jnp
import jax.experimental.pallas as pl
import jax.experimental.pallas.tpu as pltpu

H, DH, SK, W, D = 32, 128, 4096, 1024, 640
NH = 2 * H
NG = 8
PK = W // NG
DEPTH = 7
KV_PRIOS = (0, 1, 1, 1)
W_PRIO = 1
WQ_PLAN = ((4, 0, D),)
WO_PLAN = ((1, 0, 32), (3, 32, 32), (5, 64, 32), (7, 96, 32))
LAST_WO_PLAN = ((4, 0, 32), (5, 32, 32), (6, 64, 32), (7, 96, 32))
Q_G = 7
PROJ_G = 1
X_SEM = 3


def _kernel(xa, ka, va, wqa, woa, xb, kb, vb, wqb, wob, out,
            xbuf, gbuf, wqbuf, wobuf, qbuf, pbuf, lbuf, obuf, acc, gsem):
    xs, ks, vs, wqs, wos = (xa, xb), (ka, kb), (va, vb), (wqa, wqb), (woa, wob)
    scale = DH ** -0.5

    def slot_of(jpar, g):
        return jpar * NG + g

    def wq_copy(br, h, jpar, g, r0, rn):
        return pltpu.make_async_copy(
            wqs[br].at[pl.ds(r0, rn), pl.ds(pl.multiple_of(h * DH, DH), DH)],
            wqbuf.at[jpar, pl.ds(r0, rn), :], gsem.at[g])

    def wo_copy(br, h, jpar, g, r0, rn):
        return pltpu.make_async_copy(
            wos[br].at[pl.ds(pl.multiple_of(h * DH + r0, rn), rn), :],
            wobuf.at[jpar, pl.ds(r0, rn), :], gsem.at[g])

    def kv_copy(src, b, h, jpar, g, kp, which):
        return pltpu.make_async_copy(
            src.at[b, h, pl.ds(SK - W + kp * PK, PK), :], gbuf.at[slot_of(jpar, g), which], gsem.at[g])

    def kv_list(g, kj, vj):
        if kj is not None and vj is not None:
            return ([(ks[kj[0]], b, kj[1], g, b) for b in range(2)]
                    + [(vs[vj[0]], b, vj[1], g, 2 + b) for b in range(2)])
        if kj is not None:
            if g < 4:
                return []
            return ([(ks[kj[0]], b, kj[1], g - 4, b) for b in range(2)]
                    + [(ks[kj[0]], b, kj[1], g, 2 + b) for b in range(2)])
        if g >= 4:
            return []
        return ([(vs[vj[0]], b, vj[1], g, b) for b in range(2)]
                + [(vs[vj[0]], b, vj[1], g + 4, 2 + b) for b in range(2)])

    def w_copies(jpar, g, vj, qj, wop):
        ws = []
        if qj is not None:
            ws += [wq_copy(qj[0], qj[1], jpar, *e) for e in WQ_PLAN if e[0] == g]
        if vj is not None:
            ws += [wo_copy(vj[0], vj[1], jpar, *e) for e in wop if e[0] == g]
        return ws

    def start_group(jpar, g, kj, vj, qj, wop):
        for n, (src, b, h, kp, which) in enumerate(kv_list(g, kj, vj)):
            kv_copy(src, b, h, jpar, g, kp, which).start(priority=KV_PRIOS[n])
        for c in w_copies(jpar, g, vj, qj, wop):
            c.start(priority=W_PRIO)

    def wait_group(jpar, g, kj, vj, qj, wop):
        s = slot_of(jpar, g)
        if kv_list(g, kj, vj):
            pltpu.make_async_copy(gbuf.at[s], gbuf.at[s], gsem.at[g]).wait()
        for c in w_copies(jpar, g, vj, qj, wop):
            c.wait()

    def compute_q(br, sl):
        xv = xbuf[br]
        x16 = jnp.concatenate([jnp.broadcast_to(xv[0:1], (8, D)), jnp.broadcast_to(xv[1:2], (8, D))], axis=0)
        q = jnp.dot(x16, wqbuf[sl], preferred_element_type=jnp.float32)
        qbuf[...] = q.astype(jnp.bfloat16)

    def flush(br, a):
        out[0:1, br * D:(br + 1) * D] = a[0:1].astype(out.dtype)
        out[1:2, br * D:(br + 1) * D] = a[8:9].astype(out.dtype)

    def qk(q, s, which):
        return jax.lax.dot_general(q, gbuf[s, which], (((1,), (1,)), ((), ())),
                                   preferred_element_type=jnp.float32)

    def pv(p, s, which):
        return jnp.dot(p, gbuf[s, which], preferred_element_type=jnp.float32)

    def step(jpar, hk, hv, hp, hn, hnn, wop=WO_PLAN, wop_next=WO_PLAN, after_proj=None):
        first, last = hv is None, hk is None
        q = None if last else qbuf[...]
        p_prev = None if first else pbuf[...]
        s0, s1 = {}, {}
        a0 = a1 = None
        for g in range(4 if first else 0, NG):
            wait_group(jpar, g, hk, hv, hn, wop)
            n = g + DEPTH
            if n < NG:
                start_group(jpar, n, hk, hv, hn, wop)
            elif not last:
                start_group(1 - jpar, n - NG, hn, hk, hnn, wop_next)
            s = slot_of(jpar, g)
            if first:
                qk_todo, pv_todo = ((g - 4, 0), (g, 2)), ()
            elif last:
                qk_todo, pv_todo = (), (((g, 0), (g + 4, 2)) if g < 4 else ())
            else:
                qk_todo, pv_todo = ((g, 0),), ((g, 2),)
            for kp, w0 in qk_todo:
                s0[kp] = qk(q, s, w0)[0:8]
                s1[kp] = qk(q, s, w0 + 1)[8:16]
            for kp, w0 in pv_todo:
                pg = p_prev[:, kp * PK:(kp + 1) * PK]
                o0, o1 = pv(pg, s, w0)[0:8], pv(pg, s, w0 + 1)[8:16]
                a0 = o0 if a0 is None else a0 + o0
                a1 = o1 if a1 is None else a1 + o1
            if hp is not None and g == PROJ_G:
                acc[...] += jnp.dot(obuf[...], wobuf[1 - jpar], preferred_element_type=jnp.float32)
                if after_proj is not None:
                    after_proj()
            if last and g == 3:
                obuf[...] = (jnp.concatenate([a0, a1], axis=0) / lbuf[...]).astype(jnp.bfloat16)
            if hn is not None and g == Q_G:
                compute_q(hn[0], jpar)
        if last:
            return
        if not first:
            obuf[...] = (jnp.concatenate([a0, a1], axis=0) / lbuf[...]).astype(jnp.bfloat16)
        sc = jnp.concatenate([jnp.concatenate([s0[i] for i in range(NG)], axis=1),
                              jnp.concatenate([s1[i] for i in range(NG)], axis=1)], axis=0) * scale
        m = jnp.max(sc, axis=-1, keepdims=True)
        p = jnp.exp(sc - m)
        l = jnp.sum(p, axis=-1, keepdims=True)
        pbuf[...] = p.astype(jnp.bfloat16)
        lbuf[...] = jnp.broadcast_to(l, (16, DH))

    x_c = [pltpu.make_async_copy(xs[i], xbuf.at[i], gsem.at[X_SEM]) for i in range(2)]
    wq0 = pltpu.make_async_copy(wqa.at[:, pl.ds(0, DH)], wqbuf.at[1], gsem.at[X_SEM])
    x_c[0].start()
    wq0.start(priority=1)
    x_c[1].start()
    for n in range(4, 4 + DEPTH):
        if n < NG:
            start_group(0, n, (0, 0), None, (0, 1), WO_PLAN)
        else:
            start_group(1, n - NG, (0, 1), (0, 0), (0, 2), WO_PLAN)
    x_c[0].wait()
    x_c[1].wait()
    wq0.wait()
    compute_q(0, 1)
    acc[...] = jnp.zeros_like(acc)

    def run(lo, hi, br):
        def body(t, carry):
            h = lo + 2 * t
            step(0, (br, h), (br, h - 1), (br, h - 2), (br, h + 1), (br, h + 2))
            step(1, (br, h + 1), (br, h), (br, h - 1), (br, h + 2), (br, h + 3))
            return carry
        jax.lax.fori_loop(0, (hi - lo) // 2, body, 0)

    def head(j):
        return (j // H, j % H) if 0 <= j < NH else None

    def static_step(j, **kw):
        step(j % 2, head(j), head(j - 1), head(j - 2), head(j + 1), head(j + 2), **kw)

    def end_branch_a():
        flush(0, acc[...])
        acc[...] = jnp.zeros_like(acc)

    static_step(0)
    static_step(1)
    run(2, H - 2, 0)
    static_step(H - 2)
    static_step(H - 1)
    static_step(H)
    static_step(H + 1, after_proj=end_branch_a)
    run(2, H - 2, 1)
    static_step(NH - 2)
    static_step(NH - 1, wop_next=LAST_WO_PLAN)
    static_step(NH, wop=LAST_WO_PLAN)
    flush(1, acc[...] + jnp.dot(obuf[...], wobuf[NH % 2], preferred_element_type=jnp.float32))


@jax.jit
def pallas_concat_heads__sliding_block_cached__sliding_block_cached__decode_kernel(
    A_x: jax.Array,
    A_k_cache: jax.Array,
    A_v_cache: jax.Array,
    A_wq: jax.Array,
    A_wo: jax.Array,
    B_x: jax.Array,
    B_k_cache: jax.Array,
    B_v_cache: jax.Array,
    B_wq: jax.Array,
    B_wo: jax.Array,
):
    o = pl.pallas_call(
        _kernel,
        name="concat_heads_sliding_decode",
        out_shape=jax.ShapeDtypeStruct((2, 2 * D), jnp.bfloat16),
        in_specs=[pl.BlockSpec(memory_space=pl.ANY)] * 10,
        out_specs=pl.BlockSpec(memory_space=pltpu.VMEM),
        scratch_shapes=[
            pltpu.VMEM((2, 2, D), jnp.bfloat16),
            pltpu.VMEM((2 * NG, 4, PK, DH), jnp.bfloat16),
            pltpu.VMEM((2, D, DH), jnp.bfloat16),
            pltpu.VMEM((2, DH, D), jnp.bfloat16),
            pltpu.VMEM((16, DH), jnp.bfloat16),
            pltpu.VMEM((16, W), jnp.bfloat16),
            pltpu.VMEM((16, DH), jnp.float32),
            pltpu.VMEM((16, DH), jnp.bfloat16),
            pltpu.VMEM((16, D), jnp.float32),
            pltpu.SemaphoreType.DMA((NG,)),
        ],
        compiler_params=pltpu.CompilerParams(vmem_limit_bytes=32 * 1024 * 1024),
    )(A_x.reshape(2, D), A_k_cache, A_v_cache, A_wq, A_wo, B_x.reshape(2, D), B_k_cache, B_v_cache, B_wq, B_wo)
    return o.reshape(2, 1, 2 * D)
```

```python
import jax
import jax.numpy as jnp
import jax.experimental.pallas as pl
import jax.experimental.pallas.tpu as pltpu

H, DH, SK, W, D = 32, 128, 4096, 1024, 640
NH = 2 * H
NG = 8
PK = W // NG
DEPTH = 7
KV_PRIOS = (0, 1, 1, 1)
W_PRIO = 1
WQ_PLAN = ((4, 0, D),)
WO_PLAN = ((1, 0, 32), (3, 32, 32), (5, 64, 32), (7, 96, 32))
LAST_WO_PLAN = ((4, 0, 32), (5, 32, 32), (6, 64, 32), (7, 96, 32))
Q_G = 7
PROJ_G = 1
X_SEM = 3
ROT = (0, 1, 4, 5)
SHIFT = (0, 64)


def _kernel(xa, ka, va, wqa, woa, xb, kb, vb, wqb, wob, out,
            xbuf, gbuf, wqbuf, wobuf, qbuf, pbuf, lbuf, obuf, acc, gsem):
    xs, ks, vs, wqs, wos = (xa, xb), (ka, kb), (va, vb), (wqa, wqb), (woa, wob)
    scale = DH ** -0.5

    def slot_of(jpar, g):
        return jpar * NG + g

    def wq_copy(br, h, jpar, g, r0, rn):
        return pltpu.make_async_copy(
            wqs[br].at[pl.ds(r0, rn), pl.ds(pl.multiple_of(h * DH, DH), DH)],
            wqbuf.at[jpar, pl.ds(r0, rn), :], gsem.at[g])

    def wo_copy(br, h, jpar, g, r0, rn):
        return pltpu.make_async_copy(
            wos[br].at[pl.ds(pl.multiple_of(h * DH + r0, rn), rn), :],
            wobuf.at[jpar, pl.ds(r0, rn), :], gsem.at[g])

    def kv_copies(src, b, h, jpar, g, kp, which, sh):
        s = slot_of(jpar, g)
        if sh == 0 or kp < NG - 1:
            return [pltpu.make_async_copy(
                src.at[b, h, pl.ds(SK - W + sh + kp * PK, PK), :], gbuf.at[s, which], gsem.at[g])]
        return [pltpu.make_async_copy(src.at[b, h, pl.ds(SK - W, sh), :],
                                      gbuf.at[s, which, pl.ds(0, sh), :], gsem.at[g]),
                pltpu.make_async_copy(src.at[b, h, pl.ds(SK - (PK - sh), PK - sh), :],
                                      gbuf.at[s, which, pl.ds(sh, PK - sh), :], gsem.at[g])]

    def kv_list(g, kj, vj):
        if kj is not None and vj is not None:
            return ([(ks[kj[0]], b, kj[1], (g + ROT[b]) % NG, b, SHIFT[kj[0]]) for b in range(2)]
                    + [(vs[vj[0]], b, vj[1], (g + ROT[2 + b]) % NG, 2 + b, SHIFT[vj[0]]) for b in range(2)])
        if kj is not None:
            if g < 4:
                return []
            return ([(ks[kj[0]], b, kj[1], g - 4, b, SHIFT[kj[0]]) for b in range(2)]
                    + [(ks[kj[0]], b, kj[1], g, 2 + b, SHIFT[kj[0]]) for b in range(2)])
        if g >= 4:
            return []
        return ([(vs[vj[0]], b, vj[1], g, b, SHIFT[vj[0]]) for b in range(2)]
                + [(vs[vj[0]], b, vj[1], g + 4, 2 + b, SHIFT[vj[0]]) for b in range(2)])

    def w_copies(jpar, g, vj, qj, wop):
        ws = []
        if qj is not None:
            ws += [wq_copy(qj[0], qj[1], jpar, *e) for e in WQ_PLAN if e[0] == g]
        if vj is not None:
            ws += [wo_copy(vj[0], vj[1], jpar, *e) for e in wop if e[0] == g]
        return ws

    def start_group(jpar, g, kj, vj, qj, wop):
        for n, (src, b, h, kp, which, sh) in enumerate(kv_list(g, kj, vj)):
            for c in kv_copies(src, b, h, jpar, g, kp, which, sh):
                c.start(priority=KV_PRIOS[n])
        for c in w_copies(jpar, g, vj, qj, wop):
            c.start(priority=W_PRIO)

    def wait_group(jpar, g, kj, vj, qj, wop):
        s = slot_of(jpar, g)
        if kv_list(g, kj, vj):
            pltpu.make_async_copy(gbuf.at[s], gbuf.at[s], gsem.at[g]).wait()
        for c in w_copies(jpar, g, vj, qj, wop):
            c.wait()

    def compute_q(br, sl):
        xv = xbuf[br]
        x16 = jnp.concatenate([jnp.broadcast_to(xv[0:1], (8, D)), jnp.broadcast_to(xv[1:2], (8, D))], axis=0)
        q = jnp.dot(x16, wqbuf[sl], preferred_element_type=jnp.float32)
        qbuf[...] = q.astype(jnp.bfloat16)

    def flush(br, a):
        out[0:1, br * D:(br + 1) * D] = a[0:1].astype(out.dtype)
        out[1:2, br * D:(br + 1) * D] = a[8:9].astype(out.dtype)

    def qk(q, s, which):
        return jax.lax.dot_general(q, gbuf[s, which], (((1,), (1,)), ((), ())),
                                   preferred_element_type=jnp.float32)

    def pv(p, s, which):
        return jnp.dot(p, gbuf[s, which], preferred_element_type=jnp.float32)

    def step(jpar, hk, hv, hp, hn, hnn, wop=WO_PLAN, wop_next=WO_PLAN, after_proj=None):
        first, last = hv is None, hk is None
        q = None if last else qbuf[...]
        p_prev = None if first else pbuf[...]
        s0, s1 = {}, {}
        a0 = a1 = None
        for g in range(4 if first else 0, NG):
            wait_group(jpar, g, hk, hv, hn, wop)
            n = g + DEPTH
            if n < NG:
                start_group(jpar, n, hk, hv, hn, wop)
            elif not last:
                start_group(1 - jpar, n - NG, hn, hk, hnn, wop_next)
            s = slot_of(jpar, g)
            if first:
                qk_todo, pv_todo = ((g - 4, g - 4, 0), (g, g, 2)), ()
            elif last:
                qk_todo, pv_todo = (), (((g, g, 0), (g + 4, g + 4, 2)) if g < 4 else ())
            else:
                qk_todo = (((g + ROT[0]) % NG, (g + ROT[1]) % NG, 0),)
                pv_todo = (((g + ROT[2]) % NG, (g + ROT[3]) % NG, 2),)
            for k0, k1, w0 in qk_todo:
                s0[k0] = qk(q, s, w0)[0:8]
                s1[k1] = qk(q, s, w0 + 1)[8:16]
            for k0, k1, w0 in pv_todo:
                o0 = pv(p_prev[:, k0 * PK:(k0 + 1) * PK], s, w0)[0:8]
                o1 = pv(p_prev[:, k1 * PK:(k1 + 1) * PK], s, w0 + 1)[8:16]
                a0 = o0 if a0 is None else a0 + o0
                a1 = o1 if a1 is None else a1 + o1
            if hp is not None and g == PROJ_G:
                acc[...] += jnp.dot(obuf[...], wobuf[1 - jpar], preferred_element_type=jnp.float32)
                if after_proj is not None:
                    after_proj()
            if last and g == 3:
                obuf[...] = (jnp.concatenate([a0, a1], axis=0) / lbuf[...]).astype(jnp.bfloat16)
            if hn is not None and g == Q_G:
                compute_q(hn[0], jpar)
        if last:
            return
        if not first:
            obuf[...] = (jnp.concatenate([a0, a1], axis=0) / lbuf[...]).astype(jnp.bfloat16)
        sc = jnp.concatenate([jnp.concatenate([s0[i] for i in range(NG)], axis=1),
                              jnp.concatenate([s1[i] for i in range(NG)], axis=1)], axis=0) * scale
        m = jnp.max(sc, axis=-1, keepdims=True)
        p = jnp.exp(sc - m)
        l = jnp.sum(p, axis=-1, keepdims=True)
        pbuf[...] = p.astype(jnp.bfloat16)
        lbuf[...] = jnp.broadcast_to(l, (16, DH))

    x_c = [pltpu.make_async_copy(xs[i], xbuf.at[i], gsem.at[X_SEM]) for i in range(2)]
    wq0 = pltpu.make_async_copy(wqa.at[:, pl.ds(0, DH)], wqbuf.at[1], gsem.at[X_SEM])
    x_c[0].start()
    wq0.start(priority=1)
    x_c[1].start()
    for n in range(4, 4 + DEPTH):
        if n < NG:
            start_group(0, n, (0, 0), None, (0, 1), WO_PLAN)
        else:
            start_group(1, n - NG, (0, 1), (0, 0), (0, 2), WO_PLAN)
    x_c[0].wait()
    x_c[1].wait()
    wq0.wait()
    compute_q(0, 1)
    acc[...] = jnp.zeros_like(acc)

    def run(lo, hi, br):
        def body(t, carry):
            h = lo + 2 * t
            step(0, (br, h), (br, h - 1), (br, h - 2), (br, h + 1), (br, h + 2))
            step(1, (br, h + 1), (br, h), (br, h - 1), (br, h + 2), (br, h + 3))
            return carry
        jax.lax.fori_loop(0, (hi - lo) // 2, body, 0)

    def head(j):
        return (j // H, j % H) if 0 <= j < NH else None

    def static_step(j, **kw):
        step(j % 2, head(j), head(j - 1), head(j - 2), head(j + 1), head(j + 2), **kw)

    def end_branch_a():
        flush(0, acc[...])
        acc[...] = jnp.zeros_like(acc)

    static_step(0)
    static_step(1)
    run(2, H - 2, 0)
    static_step(H - 2)
    static_step(H - 1)
    static_step(H)
    static_step(H + 1, after_proj=end_branch_a)
    run(2, H - 2, 1)
    static_step(NH - 2)
    static_step(NH - 1, wop_next=LAST_WO_PLAN)
    static_step(NH, wop=LAST_WO_PLAN)
    flush(1, acc[...] + jnp.dot(obuf[...], wobuf[NH % 2], preferred_element_type=jnp.float32))


@jax.jit
def pallas_concat_heads__sliding_block_cached__sliding_block_cached__decode_kernel(
    A_x: jax.Array,
    A_k_cache: jax.Array,
    A_v_cache: jax.Array,
    A_wq: jax.Array,
    A_wo: jax.Array,
    B_x: jax.Array,
    B_k_cache: jax.Array,
    B_v_cache: jax.Array,
    B_wq: jax.Array,
    B_wo: jax.Array,
):
    o = pl.pallas_call(
        _kernel,
        name="concat_heads_sliding_decode",
        out_shape=jax.ShapeDtypeStruct((2, 2 * D), jnp.bfloat16),
        in_specs=[pl.BlockSpec(memory_space=pl.ANY)] * 10,
        out_specs=pl.BlockSpec(memory_space=pltpu.VMEM),
        scratch_shapes=[
            pltpu.VMEM((2, 2, D), jnp.bfloat16),
            pltpu.VMEM((2 * NG, 4, PK, DH), jnp.bfloat16),
            pltpu.VMEM((2, D, DH), jnp.bfloat16),
            pltpu.VMEM((2, DH, D), jnp.bfloat16),
            pltpu.VMEM((16, DH), jnp.bfloat16),
            pltpu.VMEM((16, W), jnp.bfloat16),
            pltpu.VMEM((16, DH), jnp.float32),
            pltpu.VMEM((16, DH), jnp.bfloat16),
            pltpu.VMEM((16, D), jnp.float32),
            pltpu.SemaphoreType.DMA((NG,)),
        ],
        compiler_params=pltpu.CompilerParams(vmem_limit_bytes=32 * 1024 * 1024),
    )(A_x.reshape(2, D), A_k_cache, A_v_cache, A_wq, A_wo, B_x.reshape(2, D), B_k_cache, B_v_cache, B_wq, B_wo)
    return o.reshape(2, 1, 2 * D)
```

```python
import jax
import jax.numpy as jnp
import jax.experimental.pallas as pl
import jax.experimental.pallas.tpu as pltpu

H, DH, SK, W, D = 32, 128, 4096, 1024, 640
NH = 2 * H
NG = 8
PK = W // NG
NT = D * H * DH // (8 * 128)
TPP = 16
TPH = D * DH // (8 * 128)
NPRO = NT // TPP // 4
DEPTH = 7
KV_PRIOS = (0, 1, 1, 1)
W_PRIO = 1
WQ_GROUPS = (0, 2, 4, 6, 7)
WQ_GROUPS_FIRST = (4, 5, 6, 7, 7)
WO_GROUPS = (1, 3, 5, 6, 7)
WO_GROUPS_LAST = (4, 5, 6, 7, 7)
Q_G = 5
PROJ_G = 1
ROT = (0, 1, 4, 5)
SHIFT = (0, 64)
WSHIFT = (0, 8)


def _kernel(xa, ka, va, wqa, woa, xb, kb, vb, wqb, wob, out,
            xbuf, gbuf, wqbuf, wobuf, qbuf, pbuf, lbuf, obuf, acc, gsem):
    xs, ks, vs, wqs, wos = (xa, xb), (ka, kb), (va, vb), (wqa, wqb), (woa, wob)
    scale = DH ** -0.5

    def slot_of(jpar, g):
        return jpar * NG + g

    def tiles_copy(src, s0, dst, d0, n, g):
        return pltpu.make_async_copy(src.at[pl.ds(s0, n)], dst.at[pl.ds(d0, n)], gsem.at[g])

    def wq_copies(br, i, g, is_last):
        sh = WSHIFT[br]
        dst = wqbuf.at[br]
        if sh == 0 or not is_last:
            return [tiles_copy(wqs[br], sh + i * TPP, dst, sh + i * TPP, TPP, g)]
        return [tiles_copy(wqs[br], 0, dst, 0, sh, g),
                tiles_copy(wqs[br], NT - (TPP - sh), dst, NT - (TPP - sh), TPP - sh, g)]

    def wo_copies(br, h, jpar, i, g):
        sh = WSHIFT[br]
        dst = wobuf.at[jpar]
        base = h * TPH
        if sh == 0 or i < TPH // TPP - 1:
            return [tiles_copy(wos[br], base + sh + i * TPP, dst, sh + i * TPP, TPP, g)]
        return [tiles_copy(wos[br], base, dst, 0, sh, g),
                tiles_copy(wos[br], base + TPH - (TPP - sh), dst, TPH - (TPP - sh), TPP - sh, g)]

    def kv_copies(src, b, h, jpar, g, kp, which, sh):
        s = slot_of(jpar, g)
        if sh == 0 or kp < NG - 1:
            return [pltpu.make_async_copy(
                src.at[b, h, pl.ds(SK - W + sh + kp * PK, PK), :], gbuf.at[s, which], gsem.at[g])]
        return [pltpu.make_async_copy(src.at[b, h, pl.ds(SK - W, sh), :],
                                      gbuf.at[s, which, pl.ds(0, sh), :], gsem.at[g]),
                pltpu.make_async_copy(src.at[b, h, pl.ds(SK - (PK - sh), PK - sh), :],
                                      gbuf.at[s, which, pl.ds(sh, PK - sh), :], gsem.at[g])]

    def kv_list(g, kj, vj):
        if kj is not None and vj is not None:
            return ([(ks[kj[0]], b, kj[1], (g + ROT[b]) % NG, b, SHIFT[kj[0]]) for b in range(2)]
                    + [(vs[vj[0]], b, vj[1], (g + ROT[2 + b]) % NG, 2 + b, SHIFT[vj[0]]) for b in range(2)])
        if kj is not None:
            if g < 4:
                return []
            return ([(ks[kj[0]], b, kj[1], g - 4, b, SHIFT[kj[0]]) for b in range(2)]
                    + [(ks[kj[0]], b, kj[1], g, 2 + b, SHIFT[kj[0]]) for b in range(2)])
        if g >= 4:
            return []
        return ([(vs[vj[0]], b, vj[1], g, b, SHIFT[vj[0]]) for b in range(2)]
                + [(vs[vj[0]], b, vj[1], g + 4, 2 + b, SHIFT[vj[0]]) for b in range(2)])

    def w_copies(jpar, g, kj, vj, wog, last_a):
        ws = []
        if kj is not None and kj[0] == 0:
            for n, gg in enumerate(WQ_GROUPS if vj is not None else WQ_GROUPS_FIRST):
                if gg == g:
                    ws += wq_copies(1, kj[1] * 5 + n, g, last_a and n == 4)
        if vj is not None:
            for n, gg in enumerate(wog):
                if gg == g:
                    ws += wo_copies(vj[0], vj[1], jpar, n, g)
        return ws

    def start_group(jpar, g, kj, vj, wog, last_a):
        for n, (src, b, h, kp, which, sh) in enumerate(kv_list(g, kj, vj)):
            for c in kv_copies(src, b, h, jpar, g, kp, which, sh):
                c.start(priority=KV_PRIOS[n])
        for c in w_copies(jpar, g, kj, vj, wog, last_a):
            c.start(priority=W_PRIO)

    def wait_group(jpar, g, kj, vj, wog, last_a):
        s = slot_of(jpar, g)
        if kv_list(g, kj, vj):
            pltpu.make_async_copy(gbuf.at[s], gbuf.at[s], gsem.at[g]).wait()
        for c in w_copies(jpar, g, kj, vj, wog, last_a):
            c.wait()

    def compute_q(br, h):
        xv = xbuf[br]
        x16 = jnp.concatenate([jnp.broadcast_to(xv[0:1], (8, D)), jnp.broadcast_to(xv[1:2], (8, D))], axis=0)
        wh = jnp.concatenate([wqbuf[br, H * t + h] for t in range(D // 8)], axis=0)
        q = jnp.dot(x16, wh, preferred_element_type=jnp.float32)
        qbuf[...] = q.astype(jnp.bfloat16)

    def proj(sl):
        o = obuf[...]
        return [jnp.dot(o, jnp.concatenate([wobuf[sl, (D // 128) * t + c] for t in range(DH // 8)], axis=0),
                        preferred_element_type=jnp.float32) for c in range(D // 128)]

    def flush(br, a):
        out[0:1, br * D:(br + 1) * D] = a[0:1].astype(out.dtype)
        out[1:2, br * D:(br + 1) * D] = a[8:9].astype(out.dtype)

    def qk(q, s, which):
        return jax.lax.dot_general(q, gbuf[s, which], (((1,), (1,)), ((), ())),
                                   preferred_element_type=jnp.float32)

    def pv(p, s, which):
        return jnp.dot(p, gbuf[s, which], preferred_element_type=jnp.float32)

    def step(jpar, hk, hv, hp, hn, wog=WO_GROUPS, wog_next=WO_GROUPS, after_proj=None,
             last_a=False, next_last_a=False):
        first, last = hv is None, hk is None
        q = None if last else qbuf[...]
        p_prev = None if first else pbuf[...]
        s0, s1 = {}, {}
        a0 = a1 = None
        for g in range(4 if first else 0, NG):
            wait_group(jpar, g, hk, hv, wog, last_a)
            n = g + DEPTH
            if n < NG:
                start_group(jpar, n, hk, hv, wog, last_a)
            elif not last:
                start_group(1 - jpar, n - NG, hn, hk, wog_next, next_last_a)
            s = slot_of(jpar, g)
            if first:
                qk_todo, pv_todo = ((g - 4, g - 4, 0), (g, g, 2)), ()
            elif last:
                qk_todo, pv_todo = (), (((g, g, 0), (g + 4, g + 4, 2)) if g < 4 else ())
            else:
                qk_todo = (((g + ROT[0]) % NG, (g + ROT[1]) % NG, 0),)
                pv_todo = (((g + ROT[2]) % NG, (g + ROT[3]) % NG, 2),)
            for k0, k1, w0 in qk_todo:
                s0[k0] = qk(q, s, w0)[0:8]
                s1[k1] = qk(q, s, w0 + 1)[8:16]
            for k0, k1, w0 in pv_todo:
                o0 = pv(p_prev[:, k0 * PK:(k0 + 1) * PK], s, w0)[0:8]
                o1 = pv(p_prev[:, k1 * PK:(k1 + 1) * PK], s, w0 + 1)[8:16]
                a0 = o0 if a0 is None else a0 + o0
                a1 = o1 if a1 is None else a1 + o1
            if hp is not None and g == PROJ_G:
                r = proj(1 - jpar)
                for c in range(D // 128):
                    acc[:, c * 128:(c + 1) * 128] += r[c]
                if after_proj is not None:
                    after_proj()
            if last and g == 3:
                obuf[...] = (jnp.concatenate([a0, a1], axis=0) / lbuf[...]).astype(jnp.bfloat16)
            if hn is not None and g == (NG - 1 if last_a else Q_G):
                compute_q(hn[0], hn[1])
        if last:
            return
        if not first:
            obuf[...] = (jnp.concatenate([a0, a1], axis=0) / lbuf[...]).astype(jnp.bfloat16)
        sc = jnp.concatenate([jnp.concatenate([s0[i] for i in range(NG)], axis=1),
                              jnp.concatenate([s1[i] for i in range(NG)], axis=1)], axis=0) * scale
        m = jnp.max(sc, axis=-1, keepdims=True)
        p = jnp.exp(sc - m)
        l = jnp.sum(p, axis=-1, keepdims=True)
        pbuf[...] = p.astype(jnp.bfloat16)
        lbuf[...] = jnp.broadcast_to(l, (16, DH))

    def pro_copies(w):
        g = (w + 4) % NG
        cs = [(wq_copies(0, w + n * NPRO, g, False)[0], KV_PRIOS[n]) for n in range(4)]
        if w == 0:
            cs += [(pltpu.make_async_copy(xs[i], xbuf.at[i], gsem.at[g]), 0) for i in range(2)]
        return cs

    def pro_start(w):
        if w < NPRO:
            for c, p in pro_copies(w):
                c.start(priority=p)
        else:
            n = w - NPRO + 4
            if n < NG:
                start_group(0, n, (0, 0), None, WO_GROUPS, False)
            else:
                start_group(1, n - NG, (0, 1), (0, 0), WO_GROUPS, False)

    for w in range(DEPTH):
        pro_start(w)
    for w in range(NPRO):
        for c, p in pro_copies(w):
            c.wait()
        pro_start(w + DEPTH)
    compute_q(0, 0)
    acc[...] = jnp.zeros_like(acc)

    def run(lo, hi, br):
        def body(t, carry):
            h = lo + 2 * t
            step(0, (br, h), (br, h - 1), (br, h - 2), (br, h + 1))
            step(1, (br, h + 1), (br, h), (br, h - 1), (br, h + 2))
            return carry
        jax.lax.fori_loop(0, (hi - lo) // 2, body, 0)

    def head(j):
        return (j // H, j % H) if 0 <= j < NH else None

    def static_step(j, **kw):
        step(j % 2, head(j), head(j - 1), head(j - 2), head(j + 1),
             last_a=(j == H - 1), next_last_a=(j + 1 == H - 1), **kw)

    def end_branch_a():
        flush(0, acc[...])
        acc[...] = jnp.zeros_like(acc)

    static_step(0)
    static_step(1)
    run(2, H - 2, 0)
    static_step(H - 2)
    static_step(H - 1)
    static_step(H)
    static_step(H + 1, after_proj=end_branch_a)
    run(2, H - 2, 1)
    static_step(NH - 2)
    static_step(NH - 1, wog_next=WO_GROUPS_LAST)
    static_step(NH, wog=WO_GROUPS_LAST)
    flush(1, acc[...] + jnp.concatenate(proj(NH % 2), axis=1))


def _tile_view(w):
    r, c = w.shape
    return w.reshape(r // 8, 8, c // 128, 128).transpose(0, 2, 1, 3).reshape(r * c // 1024, 8, 128)


@jax.jit
def pallas_concat_heads__sliding_block_cached__sliding_block_cached__decode_kernel(
    A_x: jax.Array,
    A_k_cache: jax.Array,
    A_v_cache: jax.Array,
    A_wq: jax.Array,
    A_wo: jax.Array,
    B_x: jax.Array,
    B_k_cache: jax.Array,
    B_v_cache: jax.Array,
    B_wq: jax.Array,
    B_wo: jax.Array,
):
    o = pl.pallas_call(
        _kernel,
        name="concat_heads_sliding_decode",
        out_shape=jax.ShapeDtypeStruct((2, 2 * D), jnp.bfloat16),
        in_specs=[pl.BlockSpec(memory_space=pl.ANY)] * 10,
        out_specs=pl.BlockSpec(memory_space=pltpu.VMEM),
        scratch_shapes=[
            pltpu.VMEM((2, 2, D), jnp.bfloat16),
            pltpu.VMEM((2 * NG, 4, PK, DH), jnp.bfloat16),
            pltpu.VMEM((2, NT, 8, 128), jnp.bfloat16),
            pltpu.VMEM((2, TPH, 8, 128), jnp.bfloat16),
            pltpu.VMEM((16, DH), jnp.bfloat16),
            pltpu.VMEM((16, W), jnp.bfloat16),
            pltpu.VMEM((16, DH), jnp.float32),
            pltpu.VMEM((16, DH), jnp.bfloat16),
            pltpu.VMEM((16, D), jnp.float32),
            pltpu.SemaphoreType.DMA((NG,)),
        ],
        compiler_params=pltpu.CompilerParams(vmem_limit_bytes=40 * 1024 * 1024),
    )(A_x.reshape(2, D), A_k_cache, A_v_cache, _tile_view(A_wq), _tile_view(A_wo),
      B_x.reshape(2, D), B_k_cache, B_v_cache, _tile_view(B_wq), _tile_view(B_wo))
    return o.reshape(2, 1, 2 * D)
```

```python
import jax
import jax.numpy as jnp
import jax.experimental.pallas as pl
import jax.experimental.pallas.tpu as pltpu

H, DH, SK, W, D = 32, 128, 4096, 1024, 640
NH = 2 * H
NG = 8
PK = W // NG
NT = D * H * DH // (8 * 128)
TPP = 16
TPH = D * DH // (8 * 128)
NPRO = NT // TPP // 4
DEPTH = 7
KV_PRIOS = (0, 1, 1, 1)
W_PRIO = 1
WQ_GROUPS = (0, 2, 4, 6, 7)
WQ_GROUPS_FIRST = (4, 5, 6, 7, 7)
WO_GROUPS = (1, 3, 5, 6, 7)
WO_GROUPS_LAST = (4, 5, 6, 7, 7)
Q_G = 5
PROJ_G = 1
ROT = (0, 1, 4, 5)
SHIFT = (0, 64)
WSHIFT = (0, 8)


def _kernel(xa, ka, va, wqa, woa, xb, kb, vb, wqb, wob, out,
            xbuf, gbuf, wqbuf, wobuf, qbuf, pbuf, lbuf, obuf, acc, gsem):
    xs, ks, vs, wqs, wos = (xa, xb), (ka, kb), (va, vb), (wqa, wqb), (woa, wob)
    scale = DH ** -0.5

    def slot_of(jpar, g):
        return jpar * NG + g

    def tiles_copy(src, s0, dst, d0, n, g):
        return pltpu.make_async_copy(src.at[pl.ds(s0, n)], dst.at[pl.ds(d0, n)], gsem.at[g])

    def wq_copies(br, i, g, is_last):
        sh = WSHIFT[br]
        dst = wqbuf.at[br]
        if sh == 0 or not is_last:
            return [tiles_copy(wqs[br], sh + i * TPP, dst, sh + i * TPP, TPP, g)]
        return [tiles_copy(wqs[br], 0, dst, 0, sh, g),
                tiles_copy(wqs[br], NT - (TPP - sh), dst, NT - (TPP - sh), TPP - sh, g)]

    def wo_copies(br, h, jpar, i, g):
        sh = WSHIFT[br]
        dst = wobuf.at[jpar]
        base = h * TPH
        if sh == 0 or i < TPH // TPP - 1:
            return [tiles_copy(wos[br], base + sh + i * TPP, dst, sh + i * TPP, TPP, g)]
        return [tiles_copy(wos[br], base, dst, 0, sh, g),
                tiles_copy(wos[br], base + TPH - (TPP - sh), dst, TPH - (TPP - sh), TPP - sh, g)]

    def kv_copies(src, b, h, jpar, g, kp, which, sh):
        s = slot_of(jpar, g)
        if sh == 0 or kp < NG - 1:
            return [pltpu.make_async_copy(
                src.at[b, h, pl.ds(SK - W + sh + kp * PK, PK), :], gbuf.at[s, which], gsem.at[g])]
        return [pltpu.make_async_copy(src.at[b, h, pl.ds(SK - W, sh), :],
                                      gbuf.at[s, which, pl.ds(0, sh), :], gsem.at[g]),
                pltpu.make_async_copy(src.at[b, h, pl.ds(SK - (PK - sh), PK - sh), :],
                                      gbuf.at[s, which, pl.ds(sh, PK - sh), :], gsem.at[g])]

    def kv_list(g, kj, vj):
        if kj is not None and vj is not None:
            return ([(ks[kj[0]], b, kj[1], (g + ROT[b]) % NG, b, SHIFT[kj[0]]) for b in range(2)]
                    + [(vs[vj[0]], b, vj[1], (g + ROT[2 + b]) % NG, 2 + b, SHIFT[vj[0]]) for b in range(2)])
        if kj is not None:
            if g < 4:
                return []
            return ([(ks[kj[0]], b, kj[1], g - 4, b, SHIFT[kj[0]]) for b in range(2)]
                    + [(ks[kj[0]], b, kj[1], g, 2 + b, SHIFT[kj[0]]) for b in range(2)])
        if g >= 4:
            return []
        return ([(vs[vj[0]], b, vj[1], g, b, SHIFT[vj[0]]) for b in range(2)]
                + [(vs[vj[0]], b, vj[1], g + 4, 2 + b, SHIFT[vj[0]]) for b in range(2)])

    def w_copies(jpar, g, kj, vj, wog, last_a):
        ws = []
        if kj is not None and kj[0] == 0:
            for n, gg in enumerate(WQ_GROUPS if vj is not None else WQ_GROUPS_FIRST):
                if gg == g:
                    ws += wq_copies(1, kj[1] * 5 + n, g, last_a and n == 4)
        if vj is not None:
            for n, gg in enumerate(wog):
                if gg == g:
                    ws += wo_copies(vj[0], vj[1], jpar, n, g)
        return ws

    def group_copies(jpar, g, kj, vj, wog, last_a):
        cs = []
        for n, (src, b, h, kp, which, sh) in enumerate(kv_list(g, kj, vj)):
            cs += [(c, KV_PRIOS[n]) for c in kv_copies(src, b, h, jpar, g, kp, which, sh)]
        return cs + [(c, W_PRIO) for c in w_copies(jpar, g, kj, vj, wog, last_a)]

    def start_group(*a):
        for c, p in group_copies(*a):
            c.start(priority=p)

    def wait_group(*a):
        for c, _ in group_copies(*a):
            c.wait()

    def compute_q(br, h):
        xv = xbuf[br]
        x16 = jnp.concatenate([jnp.broadcast_to(xv[0:1], (8, D)), jnp.broadcast_to(xv[1:2], (8, D))], axis=0)
        wh = jnp.concatenate([wqbuf[br, H * t + h] for t in range(D // 8)], axis=0)
        q = jnp.dot(x16, wh, preferred_element_type=jnp.float32)
        qbuf[...] = q.astype(jnp.bfloat16)

    def proj(sl):
        o = obuf[...]
        return [jnp.dot(o, jnp.concatenate([wobuf[sl, (D // 128) * t + c] for t in range(DH // 8)], axis=0),
                        preferred_element_type=jnp.float32) for c in range(D // 128)]

    def flush(br, a):
        out[0:1, br * D:(br + 1) * D] = a[0:1].astype(out.dtype)
        out[1:2, br * D:(br + 1) * D] = a[8:9].astype(out.dtype)

    def qk(q, s, which):
        return jax.lax.dot_general(q, gbuf[s, which], (((1,), (1,)), ((), ())),
                                   preferred_element_type=jnp.float32)

    def pv(p, s, which):
        return jnp.dot(p, gbuf[s, which], preferred_element_type=jnp.float32)

    def step(jpar, hk, hv, hp, hn, wog=WO_GROUPS, wog_next=WO_GROUPS, after_proj=None,
             last_a=False, next_last_a=False):
        first, last = hv is None, hk is None
        q = None if last else qbuf[...]
        p_prev = None if first else pbuf[...]
        s0, s1 = {}, {}
        a0 = a1 = None
        for g in range(4 if first else 0, NG):
            wait_group(jpar, g, hk, hv, wog, last_a)
            n = g + DEPTH
            if n < NG:
                start_group(jpar, n, hk, hv, wog, last_a)
            elif not last:
                start_group(1 - jpar, n - NG, hn, hk, wog_next, next_last_a)
            s = slot_of(jpar, g)
            if first:
                qk_todo, pv_todo = ((g - 4, g - 4, 0), (g, g, 2)), ()
            elif last:
                qk_todo, pv_todo = (), (((g, g, 0), (g + 4, g + 4, 2)) if g < 4 else ())
            else:
                qk_todo = (((g + ROT[0]) % NG, (g + ROT[1]) % NG, 0),)
                pv_todo = (((g + ROT[2]) % NG, (g + ROT[3]) % NG, 2),)
            for k0, k1, w0 in qk_todo:
                s0[k0] = qk(q, s, w0)[0:8]
                s1[k1] = qk(q, s, w0 + 1)[8:16]
            for k0, k1, w0 in pv_todo:
                o0 = pv(p_prev[:, k0 * PK:(k0 + 1) * PK], s, w0)[0:8]
                o1 = pv(p_prev[:, k1 * PK:(k1 + 1) * PK], s, w0 + 1)[8:16]
                a0 = o0 if a0 is None else a0 + o0
                a1 = o1 if a1 is None else a1 + o1
            if hp is not None and g == PROJ_G:
                r = proj(1 - jpar)
                for c in range(D // 128):
                    acc[:, c * 128:(c + 1) * 128] += r[c]
                if after_proj is not None:
                    after_proj()
            if last and g == 3:
                obuf[...] = (jnp.concatenate([a0, a1], axis=0) / lbuf[...]).astype(jnp.bfloat16)
            if hn is not None and g == (NG - 1 if last_a else Q_G):
                compute_q(hn[0], hn[1])
        if last:
            return
        if not first:
            obuf[...] = (jnp.concatenate([a0, a1], axis=0) / lbuf[...]).astype(jnp.bfloat16)
        sc = jnp.concatenate([jnp.concatenate([s0[i] for i in range(NG)], axis=1),
                              jnp.concatenate([s1[i] for i in range(NG)], axis=1)], axis=0) * scale
        m = jnp.max(sc, axis=-1, keepdims=True)
        p = jnp.exp(sc - m)
        l = jnp.sum(p, axis=-1, keepdims=True)
        pbuf[...] = p.astype(jnp.bfloat16)
        lbuf[...] = jnp.broadcast_to(l, (16, DH))

    def pro_copies(w):
        g = (w + 4) % NG
        cs = [(wq_copies(0, w + n * NPRO, g, False)[0], KV_PRIOS[n]) for n in range(4)]
        if w == 0:
            cs += [(pltpu.make_async_copy(xs[i], xbuf.at[i], gsem.at[g]), 0) for i in range(2)]
        return cs

    def pro_start(w):
        if w < NPRO:
            for c, p in pro_copies(w):
                c.start(priority=p)
        else:
            n = w - NPRO + 4
            if n < NG:
                start_group(0, n, (0, 0), None, WO_GROUPS, False)
            else:
                start_group(1, n - NG, (0, 1), (0, 0), WO_GROUPS, False)

    for w in range(DEPTH):
        pro_start(w)
    for w in range(NPRO):
        for c, p in pro_copies(w):
            c.wait()
        pro_start(w + DEPTH)
    compute_q(0, 0)
    acc[...] = jnp.zeros_like(acc)

    def run(lo, hi, br):
        def body(t, carry):
            h = lo + 2 * t
            step(0, (br, h), (br, h - 1), (br, h - 2), (br, h + 1))
            step(1, (br, h + 1), (br, h), (br, h - 1), (br, h + 2))
            return carry
        jax.lax.fori_loop(0, (hi - lo) // 2, body, 0)

    def head(j):
        return (j // H, j % H) if 0 <= j < NH else None

    def static_step(j, **kw):
        step(j % 2, head(j), head(j - 1), head(j - 2), head(j + 1),
             last_a=(j == H - 1), next_last_a=(j + 1 == H - 1), **kw)

    def end_branch_a():
        flush(0, acc[...])
        acc[...] = jnp.zeros_like(acc)

    static_step(0)
    static_step(1)
    run(2, H - 2, 0)
    static_step(H - 2)
    static_step(H - 1)
    static_step(H)
    static_step(H + 1, after_proj=end_branch_a)
    run(2, H - 2, 1)
    static_step(NH - 2)
    static_step(NH - 1, wog_next=WO_GROUPS_LAST)
    static_step(NH, wog=WO_GROUPS_LAST)
    flush(1, acc[...] + jnp.concatenate(proj(NH % 2), axis=1))


def _tile_view(w):
    r, c = w.shape
    return w.reshape(r // 8, 8, c // 128, 128).transpose(0, 2, 1, 3).reshape(r * c // 1024, 8, 128)


@jax.jit
def pallas_concat_heads__sliding_block_cached__sliding_block_cached__decode_kernel(
    A_x: jax.Array,
    A_k_cache: jax.Array,
    A_v_cache: jax.Array,
    A_wq: jax.Array,
    A_wo: jax.Array,
    B_x: jax.Array,
    B_k_cache: jax.Array,
    B_v_cache: jax.Array,
    B_wq: jax.Array,
    B_wo: jax.Array,
):
    o = pl.pallas_call(
        _kernel,
        name="concat_heads_sliding_decode",
        out_shape=jax.ShapeDtypeStruct((2, 2 * D), jnp.bfloat16),
        in_specs=[pl.BlockSpec(memory_space=pl.ANY)] * 10,
        out_specs=pl.BlockSpec(memory_space=pltpu.VMEM),
        scratch_shapes=[
            pltpu.VMEM((2, 2, D), jnp.bfloat16),
            pltpu.VMEM((2 * NG, 4, PK, DH), jnp.bfloat16),
            pltpu.VMEM((2, NT, 8, 128), jnp.bfloat16),
            pltpu.VMEM((2, TPH, 8, 128), jnp.bfloat16),
            pltpu.VMEM((16, DH), jnp.bfloat16),
            pltpu.VMEM((16, W), jnp.bfloat16),
            pltpu.VMEM((16, DH), jnp.float32),
            pltpu.VMEM((16, DH), jnp.bfloat16),
            pltpu.VMEM((16, D), jnp.float32),
            pltpu.SemaphoreType.DMA((NG,)),
        ],
        compiler_params=pltpu.CompilerParams(vmem_limit_bytes=40 * 1024 * 1024),
    )(A_x.reshape(2, D), A_k_cache, A_v_cache, _tile_view(A_wq), _tile_view(A_wo),
      B_x.reshape(2, D), B_k_cache, B_v_cache, _tile_view(B_wq), _tile_view(B_wo))
    return o.reshape(2, 1, 2 * D)
```
